```python
import os as _os
_os.environ.setdefault("JAX_PLATFORMS", "cpu")
import jax
import jax.numpy as jnp

def _softmax(x, axis=-1):
    return jax.nn.softmax(x, axis=axis)
def _gelu(x):
    return jax.nn.gelu(x, approximate=True)
def _silu(x):
    return jax.nn.silu(x)
def _sigmoid(x):
    return jax.nn.sigmoid(x)
def _layernorm(x, axis=-1, eps=1e-5):
    m = jnp.mean(x, axis=axis, keepdims=True)
    v = jnp.var(x, axis=axis, keepdims=True)
    return (x - m) / jnp.sqrt(v + eps)
def _scatter_add(tgt, idx, src, axis=0):
    return tgt.at[idx].add(src)
def _segment_sum(src, seg, n):
    return jax.ops.segment_sum(src, seg, n)
class _Rng:
    def __init__(self, key):
        self._k = key
    def _next(self):
        self._k, sub = jax.random.split(self._k)
        return sub
    def normal(self, shape):
        return jax.random.normal(self._next(), shape, dtype=jnp.bfloat16)
    def randint(self, lo, hi, shape):
        return jax.random.randint(self._next(), shape, lo, hi, dtype=jnp.int32)
    def uniform(self, shape, lo=0.0, hi=1.0):
        return jax.random.uniform(self._next(), shape, jnp.bfloat16, lo, hi)
    def permutation(self, n):
        return jax.random.permutation(self._next(), n)


kernel_name = 'concat_heads__gqa_block_cached__gqa_block_cached__decode'

def setup_inputs():
    _rng = _Rng(jax.random.key(int.from_bytes(__import__("os").urandom(4), "little")))
    _w = (lambda a: (lambda t: t.astype(jnp.bfloat16) if jnp.issubdtype(t.dtype, jnp.floating) else t)(jnp.asarray(a)))
    def _A_setup():
        B, Sq, D = 2, 1, 576
        Hq, Hkv, Sk, Dh = 32, 16, 4096, 128
        assert Hq % Hkv == 0, (Hq, Hkv)
        return {
            "x": _w((lambda *s: _rng.normal(s) * 0.8)(B, Sq, D)),
            "k_cache": _w((lambda *s: _rng.normal(s) * 0.8)(B, Hkv, Sk, Dh)),
            "v_cache": _w((lambda *s: _rng.normal(s) * 0.05)(B, Hkv, Sk, Dh)),
            "wq": _w((lambda *s: _rng.normal(s) * 0.8)(D, Hq * Dh) * (D ** -0.5)),
            "wo": _w((lambda *s: _rng.normal(s) * 0.05)(Hq * Dh, D) * ((Hq * Dh) ** -0.5)),
        }
    _A_in = _A_setup()

    def _B_setup():
        B, Sq, D = 2, 1, 576
        Hq, Hkv, Sk, Dh = 32, 16, 4096, 128
        assert Hq % Hkv == 0, (Hq, Hkv)
        return {
            "x": _w((lambda *s: _rng.normal(s) * 0.8)(B, Sq, D)),
            "k_cache": _w((lambda *s: _rng.normal(s) * 0.8)(B, Hkv, Sk, Dh)),
            "v_cache": _w((lambda *s: _rng.normal(s) * 0.05)(B, Hkv, Sk, Dh)),
            "wq": _w((lambda *s: _rng.normal(s) * 0.8)(D, Hq * Dh) * (D ** -0.5)),
            "wo": _w((lambda *s: _rng.normal(s) * 0.05)(Hq * Dh, D) * ((Hq * Dh) ** -0.5)),
        }
    _B_in = _B_setup()

    return {
        "A_x": _A_in["x"],
        "A_k_cache": _A_in["k_cache"],
        "A_v_cache": _A_in["v_cache"],
        "A_wq": _A_in["wq"],
        "A_wo": _A_in["wo"],
        "B_x": _B_in["x"],
        "B_k_cache": _B_in["k_cache"],
        "B_v_cache": _B_in["v_cache"],
        "B_wq": _B_in["wq"],
        "B_wo": _B_in["wo"],
    }

def reference(A_x, A_k_cache, A_v_cache, A_wq, A_wo, B_x, B_k_cache, B_v_cache, B_wq, B_wo):
    def _A_ref(x, k_cache, v_cache, wq, wo):
        B, Sq, D = x.shape
        Hq, Dh = 32, 128
        Hkv = k_cache.shape[1]
        rep = Hq // Hkv
        q = (lambda x, *d: x.transpose(*d))((x @ wq).reshape(B, Sq, Hq, Dh), 0, 2, 1, 3)
        k = jnp.repeat(k_cache, rep, axis=1)
        v = jnp.repeat(v_cache, rep, axis=1)
        scores = jnp.einsum("bhqd,bhkd->bhqk", q, k) * (Dh ** -0.5)
        p = _softmax(scores, axis=-1)
        o = jnp.einsum("bhqk,bhkd->bhqd", p, v)
        return (lambda x, *d: x.transpose(*d))(o, 0, 2, 1, 3).reshape(B, Sq, Hq * Dh) @ wo

    def _B_ref(x, k_cache, v_cache, wq, wo):
        B, Sq, D = x.shape
        Hq, Dh = 32, 128
        Hkv = k_cache.shape[1]
        rep = Hq // Hkv
        q = (lambda x, *d: x.transpose(*d))((x @ wq).reshape(B, Sq, Hq, Dh), 0, 2, 1, 3)
        k = jnp.repeat(k_cache, rep, axis=1)
        v = jnp.repeat(v_cache, rep, axis=1)
        scores = jnp.einsum("bhqd,bhkd->bhqk", q, k) * (Dh ** -0.5)
        p = _softmax(scores, axis=-1)
        o = jnp.einsum("bhqk,bhkd->bhqd", p, v)
        return (lambda x, *d: x.transpose(*d))(o, 0, 2, 1, 3).reshape(B, Sq, Hq * Dh) @ wo

    a = _A_ref(A_x, A_k_cache, A_v_cache, A_wq, A_wo)
    b = _B_ref(B_x, B_k_cache, B_v_cache, B_wq, B_wo)
    return jnp.concatenate([a, b], axis=-1)
```

```python
import functools
import jax
import jax.numpy as jnp
from jax import lax
import jax.experimental.pallas as pl
import jax.experimental.pallas.tpu as pltpu

BF, F32 = jnp.bfloat16, jnp.float32
NT = (((1,), (1,)), ((), ()))
B, D, HKV, SK, DH = 2, 576, 16, 4096, 128
HG = 4
NU = HG * B
RPB = HKV // HG
WC = HG * 2 * DH
CH = 128


def build(depth=4, sr=512, wrows=16, compute=True):
    ns = SK // sr
    per = 2 * ns + 2
    nrounds = 2 * RPB
    total = nrounds * per
    c2 = (DH ** -0.5) * 1.4426950408889634

    def kern(xa, ka, va, wqa, woa, xb, kb, vb, wqb, wob, o_ref,
             kv, wq, wo, xs, q_s, s_s, m_s, l_s, acc_s, out_s, sems, xsem):
        hbm = ((ka, va, wqa, woa), (kb, vb, wqb, wob))

        def start_w(src, dst, g, sem):
            n = D // wrows
            nst = 9 if n % 9 == 0 else 1
            c0 = g * WC if isinstance(g, int) else pl.multiple_of(g * WC, WC)
            for i in range(n):
                r = ((i % nst) * (n // nst) + i // nst) * wrows
                pltpu.make_async_copy(src.at[pl.ds(r, wrows), pl.ds(c0, WC)],
                                      dst.at[pl.ds(r, wrows)], sem).start(priority=i % 2)

        def start_kv(src, g, j, slot, sem):
            for c in range(sr // CH):
                r0 = j * sr + c * CH
                r0 = r0 if isinstance(r0, int) else pl.multiple_of(r0, CH)
                for u in range(NU):
                    hh, b = u // B, u % B
                    pltpu.make_async_copy(src.at[b, g * HG + hh, pl.ds(r0, CH)],
                                          kv.at[slot, u, pl.ds(c * CH, CH)], sem).start(priority=u % 2)

        def start(rnd, k, slot):
            sem = sems.at[slot]
            if isinstance(rnd, int):
                kk, vv, wqq, woo = hbm[rnd // RPB]
                g = rnd % RPB
                if k == 0: start_w(wqq, wq, g, sem)
                elif k <= ns: start_kv(kk, g, k - 1, slot, sem)
                elif k <= 2 * ns: start_kv(vv, g, k - 1 - ns, slot, sem)
                else: start_w(woo, wo, g, sem)
                return
            for br in range(2):
                kk, vv, wqq, woo = hbm[br]

                @pl.when(rnd // RPB == br)
                def _():
                    g = rnd - br * RPB
                    pl.when(k == 0)(lambda: start_w(wqq, wq, g, sem))
                    pl.when((k >= 1) & (k <= ns))(lambda: start_kv(kk, g, k - 1, slot, sem))
                    pl.when((k > ns) & (k <= 2 * ns))(lambda: start_kv(vv, g, k - 1 - ns, slot, sem))
                    pl.when(k == 2 * ns + 1)(lambda: start_w(woo, wo, g, sem))

        def wait(dst, slot):
            pltpu.make_async_copy(dst, dst, sems.at[slot]).wait()

        xcp = [pltpu.make_async_copy(x, xs.at[i], xsem.at[i]) for i, x in enumerate((xa, xb))]
        for c in xcp:
            c.start()
        for t in range(depth):
            start(t // per, t % per, t)
        for c in xcp:
            c.wait()
        out_s[...] = jnp.zeros(out_s.shape, F32)

        row = lax.broadcasted_iota(jnp.int32, (8, DH), 0)

        def q_step(rnd, slot):
            wait(wq, slot)
            if not compute: return
            x = xs[rnd // RPB].astype(F32)
            xrow = lax.broadcasted_iota(jnp.int32, (8, D), 0)
            x8 = jnp.where(xrow % 2 == 0, x[0:1], x[1:2]).astype(BF)
            q = jnp.dot(x8, wq[...], preferred_element_type=F32)
            for gi in range(HG // 2):
                blk = [q[:, (gi * 4 + i) * DH:(gi * 4 + i + 1) * DH] for i in range(4)]
                qg = jnp.where(row < 4, jnp.where(row < 2, blk[0], blk[1]),
                               jnp.where(row < 6, blk[2], blk[3]))
                for ul in range(4):
                    mine = (row // 4 == ul // 2) & (row % 2 == ul % 2)
                    q_s[gi * 4 + ul] = jnp.where(mine, qg, 0.0)
            m_s[...] = jnp.full(m_s.shape, -jnp.inf, F32)
            l_s[...] = jnp.zeros(l_s.shape, F32)
            acc_s[...] = jnp.zeros(acc_s.shape, F32)

        def k_step(j, slot):
            wait(kv.at[slot], slot)
            if not compute: return
            for gi in range(HG // 2):
                s = None
                for ul in range(4):
                    u = gi * 4 + ul
                    d = lax.dot_general(q_s[u].astype(BF), kv[slot, u], NT, preferred_element_type=F32)
                    s = d if s is None else s + d
                s_s[j, gi] = s
                m = m_s[gi]
                for c in range(sr // DH):
                    m = jnp.maximum(m, s[:, c * DH:(c + 1) * DH])
                m_s[gi] = m

            @pl.when(j == ns - 1)
            def _():
                for gi in range(HG // 2):
                    m_s[gi] = jnp.broadcast_to(jnp.max(m_s[gi], axis=1, keepdims=True), (8, DH))

        def v_step(j, slot):
            wait(kv.at[slot], slot)
            if not compute: return
            for gi in range(HG // 2):
                m = m_s[gi]
                l = l_s[gi]
                ps = []
                for c in range(sr // DH):
                    p = jnp.exp2((s_s[j, gi, :, c * DH:(c + 1) * DH] - m) * c2)
                    l = l + p
                    ps.append(p)
                l_s[gi] = l
                p = jnp.concatenate(ps, axis=1).astype(BF)
                for ul in range(4):
                    u = gi * 4 + ul
                    acc_s[u] += jnp.dot(p, kv[slot, u], preferred_element_type=F32)

        def o_step(rnd, slot):
            if not compute:
                wait(wo, slot); return
            blks = []
            for gi in range(HG // 2):
                a = [acc_s[gi * 4 + ul] for ul in range(4)]
                og = jnp.where(row < 4, jnp.where(row % 2 == 0, a[0], a[1]),
                               jnp.where(row % 2 == 0, a[2], a[3]))
                og = og / jnp.sum(l_s[gi], axis=1, keepdims=True)
                for i in range(4):
                    blks.append(og if i == 0 else pltpu.roll(og, 8 - 2 * i, 0))
            o = jnp.concatenate(blks, axis=1).astype(BF)
            wait(wo, slot)
            out_s[rnd // RPB] += lax.dot_general(o, wo[...], NT, preferred_element_type=F32)

        def body(t, carry):
            rnd, k, slot, rn2, k2 = carry
            pl.when(k == 0)(lambda: q_step(rnd, slot))
            pl.when((k >= 1) & (k <= ns))(lambda: k_step(k - 1, slot))
            pl.when((k > ns) & (k <= 2 * ns))(lambda: v_step(k - 1 - ns, slot))
            pl.when(k == 2 * ns + 1)(lambda: o_step(rnd, slot))
            start(rn2, k2, slot)
            nxt = lambda r, s: (jnp.where(s == per - 1, r + 1, r), jnp.where(s == per - 1, 0, s + 1))
            return (*nxt(rnd, k), jnp.where(slot == depth - 1, 0, slot + 1), *nxt(rn2, k2))

        z = jnp.int32(0)
        lax.fori_loop(0, total, body, (z, z, z, z + depth // per, z + depth % per))
        o_ref[...] = jnp.concatenate([out_s[0, 0:2], out_s[1, 0:2]], axis=1).astype(BF)

    def f(xa, ka, va, wqa, woa, xb, kb, vb, wqb, wob):
        out = pl.pallas_call(
            kern,
            in_specs=[pl.BlockSpec(memory_space=pltpu.HBM)] * 10,
            out_shape=jax.ShapeDtypeStruct((B, 2 * D), BF),
            scratch_shapes=[
                pltpu.VMEM((depth, NU, sr, DH), BF), pltpu.VMEM((D, WC), BF), pltpu.VMEM((D, WC), BF),
                pltpu.VMEM((2, B, D), BF), pltpu.VMEM((NU, 8, DH), F32),
                pltpu.VMEM((ns, HG // 2, 8, sr), F32), pltpu.VMEM((HG // 2, 8, DH), F32),
                pltpu.VMEM((HG // 2, 8, DH), F32), pltpu.VMEM((NU, 8, DH), F32),
                pltpu.VMEM((2, 8, D), F32),
                pltpu.SemaphoreType.DMA((depth,)), pltpu.SemaphoreType.DMA((2,)),
            ],
            compiler_params=pltpu.CompilerParams(vmem_limit_bytes=64 * 1024 * 1024,
                                                 disable_bounds_checks=True),
        )(xa.reshape(B, D), ka, va, wqa, woa.T, xb.reshape(B, D), kb, vb, wqb, wob.T)
        return out.reshape(B, 1, 2 * D)
    return f


@jax.jit
def pallas_concat_heads__gqa_block_cached__gqa_block_cached__decode_kernel(
    A_x, A_k_cache, A_v_cache, A_wq, A_wo, B_x, B_k_cache, B_v_cache, B_wq, B_wo):
    return build()(A_x, A_k_cache, A_v_cache, A_wq, A_wo, B_x, B_k_cache, B_v_cache, B_wq, B_wo)
```

```python
import math

import jax
import jax.numpy as jnp
from jax import lax
import jax.experimental.pallas as pl
import jax.experimental.pallas.tpu as pltpu

BF16, F32 = jnp.bfloat16, jnp.float32
NT = (((1,), (1,)), ((), ()))

B, D, HKV, SK, DH = 2, 576, 16, 4096, 128
W = 2 * HKV * DH
QW, HW = W // 4, W // 2
NB = D // 8
FULL = D // 128
CH = 128
NS = SK // CH
NG = HKV * B // 4
DEPTH = 4
TAIL = 40
PHASE = (1, 0)
SCALE_LOG2E = DH ** -0.5 * math.log2(math.e)


def _loop(n, fn):
    lax.fori_loop(0, n, lambda i, c: (fn(i), c)[1], 0)


def _per_branch(br, fn):
    pl.when(br == 0)(lambda: fn(0))
    pl.when(br == 1)(lambda: fn(1))


def _divmod(i, d):
    q = i >> (d.bit_length() - 1) if d & (d - 1) == 0 else (i * ((1 << 20) // d + 1)) >> 20
    return q, i - q * d


def _walk(i, n, stride):
    g = math.gcd(n, stride)
    q, r = _divmod(i, n // g)
    return (r * stride if g == stride else _divmod(r * stride, n)[1]) + q


def _wait_filled(dst, sem):
    pltpu.make_async_copy(dst, dst, sem).wait()


def _kernel(xa, ka, va, wqa, woa, xb, kb, vb, wqb, wob, out_hbm,
            kv, wq, wo, xs, x8_s, q_s, s_s, m_s, l_s, acc_s, o_s, res_s, rem_s, out_s,
            kv_sem, wq_sem, wo_sem, io_sem):
    hbm = ((kb, vb, wqb, wob), (ka, va, wqa, woa))

    def start_bands(src, dst, phase, half, lo, n, band, sem_of, queues=(0, 1)):
        def copy(bnd, c_src, c_dst, width, p):
            rows = pl.ds(pl.multiple_of(bnd * 8, 8), 8)
            pltpu.make_async_copy(src.at[rows, pl.ds(c_src, width)], dst.at[rows, pl.ds(c_dst, width)],
                                  sem_of(bnd)).start(priority=queues[p])

        def pair(i):
            bnd = [band(lo + 2 * i + p) for p in range(2)]
            if phase == 0 or half == 0:
                for p in range(2):
                    copy(bnd[p], half * HW + phase * QW, half * HW, HW, p)
            else:
                for p in range(2):
                    copy(bnd[p], 3 * QW, 2 * QW, QW, p)
                for p in range(2):
                    copy(jnp.where(bnd[p] == NB - 1, 0, bnd[p] + 1), 0, 3 * QW, QW, p)
        _loop(n // 2, pair)

    def any_order(br, half):
        return lambda i: _walk(i, NB, 48 if PHASE[br] and half else 8)

    def start_wq(br, half, lo, n):
        start_bands(hbm[br][2], wq, PHASE[br], half, lo, n, any_order(br, half), lambda bnd: wq_sem.at[half])

    def start_wo(br, part):
        src, phase = hbm[br][3], PHASE[br]

        def second_half(lo, n, band, queues=(0, 1)):
            start_bands(src, wo, phase, 1, lo, n, band, lambda bnd: wo_sem.at[1 + (bnd >> 4)], queues)

        def by_block(i):
            return jnp.where(i < 16 * FULL, (i & ~15) + _walk(i & 15, 16, 12), i)

        pl.when(part < 2)(lambda: start_bands(src, wo, phase, 0, part * (NB // 2), NB // 2,
                                              any_order(br, 0), lambda bnd: wo_sem.at[0]))
        if br == 0:
            pl.when(part >= 2)(lambda: second_half((part - 2) * (NB // 2), NB // 2, any_order(br, 1)))
        else:
            pl.when(part == 2)(lambda: second_half(0, NB - TAIL, by_block))
            pl.when(part == 3)(lambda: second_half(NB - TAIL, TAIL, by_block, (1, 1)))

    def start_kv(br, which, step, slot):
        src, shift = hbm[br][which], PHASE[br] * (CH // 2)
        first = ((step >> 3) - 4 * (step & 7)) & (NS - 1)
        chunk = (first, (first - 4) & (NS - 1))
        head0 = (0, (first - 4) >> 5)
        row0 = [pl.multiple_of(c * CH + shift, CH // 2) for c in chunk]

        def copy(b, h, r_src, r_dst, n):
            pltpu.make_async_copy(src.at[b, h, pl.ds(r_src, n)], kv.at[slot, h * B + b, pl.ds(r_dst, n)],
                                  kv_sem.at[slot]).start(priority=b)

        def plain(i):
            for b in range(B):
                copy(b, (i + head0[b]) & (HKV - 1), row0[b], 0, CH)

        def general(i):
            for b in range(B):
                h = (i + head0[b]) & (HKV - 1)

                def wrapped():
                    copy(b, h, SK - shift, 0, shift)
                    copy(b, (h + 1) & (HKV - 1), 0, shift, shift)
                lax.cond(chunk[b] < NS - 1, lambda: copy(b, h, row0[b], 0, CH), wrapped)

        if shift:
            lax.cond((chunk[0] < NS - 1) & (chunk[1] < NS - 1),
                     lambda: _loop(HKV, plain), lambda: _loop(HKV, general))
        else:
            _loop(HKV, plain)

    def start_next_wq(br, part):
        @pl.when(br == 0)
        def _():
            pl.when(part < 3)(lambda: start_wq(1, 0, part * (NB // 3), NB // 3))
            pl.when(part >= 3)(lambda: start_wq(1, 1, (part - 3) * (NB // 3), NB // 3))

    start_wq(0, 0, 0, NB)
    x_copies = [pltpu.make_async_copy(x, xs.at[i], io_sem.at[i]) for i, x in enumerate((xb, xa))]
    for i, c in enumerate(x_copies):
        c.start(priority=i)
    start_wq(0, 1, 0, NB)
    for c in x_copies:
        c.wait()

    row = lax.broadcasted_iota(jnp.int32, (8, DH), 0)
    head_a, batch_a = row < 4, (row & 1) == 0

    def own_rows(a):
        return jnp.where(head_a, jnp.where(batch_a, a[0], a[1]), jnp.where(batch_a, a[2], a[3]))

    def group_of(br, quarter):
        return ((quarter + jnp.where(br == 0, PHASE[0], PHASE[1])) & 3) * 2

    def quarter_of(ref, i):
        return ref[:, pl.ds(pl.multiple_of(i * QW, QW), QW)]

    def q_quarter(br, i):
        pl.when(i == 0)(lambda: _wait_filled(wq.at[:, pl.ds(0, HW)], wq_sem.at[0]))
        pl.when(i == 2)(lambda: _wait_filled(wq.at[:, pl.ds(HW, HW)], wq_sem.at[1]))
        q = jnp.dot(x8_s[...].astype(BF16), quarter_of(wq, i), preferred_element_type=F32)
        for g in range(2):
            blk = [q[:, (4 * g + n) * DH:(4 * g + n + 1) * DH] for n in range(4)]
            q_s[group_of(br, i) + g] = jnp.where(head_a, jnp.where(row < 2, blk[0], blk[1]),
                                                 jnp.where(row < 6, blk[2], blk[3]))
        _per_branch(br, lambda b: start_kv(b, 0, i, i))

    def k_step(step, slot):
        for g in range(NG):
            q = q_s[g].astype(BF16)
            s = own_rows([lax.dot_general(q, kv[slot, 4 * g + u], NT, preferred_element_type=F32)
                          for u in range(4)])
            s_s[step, g] = s
            m_s[g] = jnp.maximum(m_s[g], s)

    def row_max():
        for g in range(NG):
            m_s[g] = jnp.broadcast_to(jnp.max(m_s[g], axis=1, keepdims=True), (8, DH))

    def v_step(step, slot):
        for g in range(NG):
            p = jnp.exp2((s_s[step, g] - m_s[g]) * SCALE_LOG2E)
            l_s[g] += p
            p = p.astype(BF16)
            acc_s[g] += own_rows([jnp.dot(p, kv[slot, 4 * g + u], preferred_element_type=F32)
                                  for u in range(4)])

    def kv_step(br, t):
        slot = t & (DEPTH - 1)
        _wait_filled(kv.at[slot], kv_sem.at[slot])
        pl.when(t < NS)(lambda: k_step(t, slot))
        pl.when(t == NS)(row_max)
        pl.when(t >= NS)(lambda: v_step(t - NS, slot))
        n = t + DEPTH

        def refill(b):
            pl.when(n < NS)(lambda: start_kv(b, 0, n, slot))
            pl.when((n >= NS) & (n < 2 * NS))(lambda: start_kv(b, 1, n - NS, slot))
            pl.when(n >= 2 * NS)(lambda: start_wo(b, n - 2 * NS))
        _per_branch(br, refill)

    def o_quarter(br, i):
        d = lax.dot_general(o_s[i].astype(BF16), quarter_of(wo, i), NT, preferred_element_type=F32)
        for n in range(FULL):
            res_s[n] += d[:, n * 128:(n + 1) * 128]
        rem_s[...] += d[:, FULL * 128:]
        start_next_wq(br, i)

    def o_second_half(rows, block):
        _wait_filled(wo.at[rows, pl.ds(HW, HW)], wo_sem.at[1 + block])
        o = jnp.concatenate([o_s[2], o_s[3]], axis=1).astype(BF16)
        return lax.dot_general(o, wo[rows, pl.ds(HW, HW)], NT, preferred_element_type=F32)

    def o_block(br, n):
        res_s[n] += o_second_half(pl.ds(pl.multiple_of(n * 128, 128), 128), n)
        start_next_wq(br, n + 2)

    def branch(br):
        x = xs[br].astype(F32)
        x_row = lax.broadcasted_iota(jnp.int32, (8, D), 0)
        x8_s[...] = jnp.where((x_row & 1) == 0, x[0:1], x[1:2])
        m_s[...] = jnp.full(m_s.shape, -jnp.inf, F32)
        for ref in (l_s, acc_s, res_s, rem_s):
            ref[...] = jnp.zeros(ref.shape, F32)

        _loop(4, lambda i: q_quarter(br, i))
        _loop(2 * NS, lambda t: kv_step(br, t))

        for i in range(4):
            heads = []
            for g in range(2):
                grp = group_of(br, i) + g
                o = acc_s[grp] / jnp.sum(l_s[grp], axis=1, keepdims=True)
                heads += [o] + [pltpu.roll(o, 8 - 2 * n, 0) for n in range(1, 4)]
            o_s[i] = jnp.concatenate(heads, axis=1)

        _wait_filled(wo.at[:, pl.ds(0, HW)], wo_sem.at[0])
        _loop(2, lambda i: o_quarter(br, i))
        _loop(FULL, lambda n: o_block(br, n))
        for n in range(FULL):
            out_s[:, n * 128:(n + 1) * 128] = res_s[n, 0:B].astype(BF16)
        rem = rem_s[...] + o_second_half(pl.ds(FULL * 128, D - FULL * 128), FULL)
        out_s[:, FULL * 128:D] = rem[0:B].astype(BF16)

        @pl.when(br == 0)
        def _():
            out_s[:, D:] = out_s[:, :D]

    _loop(2, branch)
    out_copy = pltpu.make_async_copy(out_s, out_hbm, io_sem.at[2])
    out_copy.start(priority=1)
    out_copy.wait()


@jax.jit
def pallas_concat_heads__gqa_block_cached__gqa_block_cached__decode_kernel(
    A_x: jax.Array,
    A_k_cache: jax.Array,
    A_v_cache: jax.Array,
    A_wq: jax.Array,
    A_wo: jax.Array,
    B_x: jax.Array,
    B_k_cache: jax.Array,
    B_v_cache: jax.Array,
    B_wq: jax.Array,
    B_wo: jax.Array,
):
    assert A_k_cache.shape == B_k_cache.shape == (B, HKV, SK, DH)
    assert A_wq.shape == B_wq.shape == (D, W)
    vmem, dma = pltpu.VMEM, pltpu.SemaphoreType.DMA
    out = pl.pallas_call(
        _kernel,
        in_specs=[pl.BlockSpec(memory_space=pltpu.HBM)] * 10,
        out_specs=pl.BlockSpec(memory_space=pltpu.HBM),
        out_shape=jax.ShapeDtypeStruct((B, 2 * D), BF16),
        scratch_shapes=[
            vmem((DEPTH, HKV * B, CH, DH), BF16),
            vmem((D, W), BF16),
            vmem((D, W), BF16),
            vmem((2, B, D), BF16),
            vmem((8, D), F32),
            vmem((NG, 8, DH), F32),
            vmem((NS, NG, 8, CH), F32),
            vmem((NG, 8, CH), F32),
            vmem((NG, 8, CH), F32),
            vmem((NG, 8, DH), F32),
            vmem((4, 8, QW), F32),
            vmem((FULL, 8, 128), F32),
            vmem((8, D - FULL * 128), F32),
            vmem((B, 2 * D), BF16),
            dma((DEPTH,)), dma((2,)), dma((FULL + 2,)), dma((3,)),
        ],
        compiler_params=pltpu.CompilerParams(
            vmem_limit_bytes=32 * 1024 * 1024,
            disable_bounds_checks=True,
            disable_semaphore_checks=True,
        ),
    )(A_x.reshape(B, D), A_k_cache, A_v_cache, A_wq, A_wo.T,
      B_x.reshape(B, D), B_k_cache, B_v_cache, B_wq, B_wo.T)
    return out.reshape(B, 1, 2 * D)
```
